```python
import os as _os
_os.environ.setdefault("JAX_PLATFORMS", "cpu")
import jax
import jax.numpy as jnp

def _softmax(x, axis=-1):
    return jax.nn.softmax(x, axis=axis)
def _gelu(x):
    return jax.nn.gelu(x, approximate=True)
def _silu(x):
    return jax.nn.silu(x)
def _sigmoid(x):
    return jax.nn.sigmoid(x)
def _layernorm(x, axis=-1, eps=1e-5):
    m = jnp.mean(x, axis=axis, keepdims=True)
    v = jnp.var(x, axis=axis, keepdims=True)
    return (x - m) / jnp.sqrt(v + eps)
def _scatter_add(tgt, idx, src, axis=0):
    return tgt.at[idx].add(src)
def _segment_sum(src, seg, n):
    return jax.ops.segment_sum(src, seg, n)
class _Rng:
    def __init__(self, key):
        self._k = key
    def _next(self):
        self._k, sub = jax.random.split(self._k)
        return sub
    def normal(self, shape):
        return jax.random.normal(self._next(), shape, dtype=jnp.bfloat16)
    def randint(self, lo, hi, shape):
        return jax.random.randint(self._next(), shape, lo, hi, dtype=jnp.int32)
    def uniform(self, shape, lo=0.0, hi=1.0):
        return jax.random.uniform(self._next(), shape, jnp.bfloat16, lo, hi)
    def permutation(self, n):
        return jax.random.permutation(self._next(), n)


kernel_name = 'sequential_preLN__softmax_full_mha__dense_activation_squared_relu__prompt'

def setup_inputs():
    _rng = _Rng(jax.random.key(int.from_bytes(__import__("os").urandom(4), "little")))
    _w = (lambda a: (lambda t: t.astype(jnp.bfloat16) if jnp.issubdtype(t.dtype, jnp.floating) else t)(jnp.asarray(a)))
    def _A_setup():
        B, S, D = 1, 2048, 640
        return {
            "x": _w((lambda *s: _rng.normal(s) * 0.05)(B, S, D)),
            "wqkv": _w((lambda *s: _rng.normal(s) * 0.05)(D, 3 * D)),
            "wo": _w((lambda *s: _rng.normal(s) * 0.05)(D, D)),
        }
    _A_in = _A_setup()

    def _B_setup():
        B, S, D, F = 1, 2048, 640, 1536
        return {
            "x": _w((lambda *s: _rng.normal(s) * 0.05)(B, S, D)),
            "w1": _w((lambda *s: _rng.normal(s) * 0.05)(D, F)),
            "b1": _w((lambda *s: _rng.normal(s) * 0.05)(F)),
            "w2": _w((lambda *s: _rng.normal(s) * 0.05)(F, D)),
            "b2": _w((lambda *s: _rng.normal(s) * 0.05)(D)),
        }
    _B_in = _B_setup()

    return {
        "A_x": _A_in["x"],
        "A_wqkv": _A_in["wqkv"],
        "A_wo": _A_in["wo"],
        "B_x": _B_in["x"],
        "B_w1": _B_in["w1"],
        "B_b1": _B_in["b1"],
        "B_w2": _B_in["w2"],
        "B_b2": _B_in["b2"],
    }

def reference(A_x, A_wqkv, A_wo, B_x, B_w1, B_b1, B_w2, B_b2):
    def _A_ref(x, wqkv, wo):
        B, S, D = x.shape
        H = 32; Dh = D // H
        qkv = (lambda x, *d: x.transpose(*d))((x @ wqkv).reshape(B, S, 3, H, Dh), 2, 0, 3, 1, 4)
        q, k, v = qkv[0], qkv[1], qkv[2]
        scale = Dh ** -0.5
        scores = jnp.einsum("bhqd,bhkd->bhqk", q, k) * scale
        p = _softmax(scores, axis=-1)
        o = jnp.einsum("bhqk,bhkd->bhqd", p, v)
        return (lambda x, *d: x.transpose(*d))(o, 0, 2, 1, 3).reshape(B, S, D) @ wo

    def _B_ref(x, w1, b1, w2, b2):
        h = jnp.einsum("bsd,df->bsf", x, w1) + b1
        zero = jnp.zeros_like(h)
        r = jnp.where(h > zero, h, zero)
        h = r * r
        out = jnp.einsum("bsf,fd->bsd", h, w2) + b2
        return out

    x = A_x
    h = x + _A_ref(_layernorm(x, axis=-1), A_wqkv, A_wo)
    h2 = h + _B_ref(_layernorm(h, axis=-1), B_w1, B_b1, B_w2, B_b2)
    return h2
```

```python
import functools
import math

import jax
import jax.numpy as jnp
from jax import lax
import jax.experimental.pallas as pl
import jax.experimental.pallas.tpu as pltpu

F32 = jnp.float32
BF16 = jnp.bfloat16

N_HEADS = 32
TOK = 512
KEY_BLK = 128
PAIRS_PER_STEP = 4
LAG = 2

SCORE_BOUND = 64.0
GRID = 2.0 ** -7
HI_SCALE = 2.0 * SCORE_BOUND / GRID
BIG = 1.5 * 2.0 ** 23 * GRID * HI_SCALE


def _dot(a, b):
    return lax.dot_general(a, b, (((1,), (0,)), ((), ())), preferred_element_type=F32)


def _layernorm_t(x):
    n = x.shape[0]
    mean = jnp.sum(x, axis=0, keepdims=True) * (1.0 / n)
    xc = x - mean
    var = jnp.sum(xc * xc, axis=0, keepdims=True) * (1.0 / n)
    return xc * lax.rsqrt(var + 1e-5)


def _kernel(x_hbm, wqkv_hbm, wo_hbm, w1_hbm, b1_ref, w2_hbm, b2_ref, out_hbm,
            x_v, wqkv_v, wo_v, w1_v, w2_v,
            xt_s, wqkvt_s, wot_s, w1t_s, w2t_s,
            k_s, q_s, v_s, ot_s, out_v, in_sem, out_sem, *, seq, dim, dh):
    n_tiles = seq // TOK
    n_pairs = N_HEADS // 2
    pr = 2 * dh
    q_scale = dh ** -0.5 * math.log2(math.e)

    x_cp = [pltpu.make_async_copy(x_hbm.at[0, pl.ds(i * TOK, TOK), :],
                                  x_v.at[pl.ds(i * TOK, TOK), :], in_sem.at[i])
            for i in range(n_tiles)]
    wqkv_cp = [pltpu.make_async_copy(wqkv_hbm.at[:, pl.ds(j * dim, dim)],
                                     wqkv_v.at[:, pl.ds(j * dim, dim)], in_sem.at[n_tiles + j])
               for j in range(3)]
    wo_cp = pltpu.make_async_copy(wo_hbm, wo_v, in_sem.at[n_tiles + 3])
    w1_cp = pltpu.make_async_copy(w1_hbm, w1_v, in_sem.at[n_tiles + 4])
    w2_cp = pltpu.make_async_copy(w2_hbm, w2_v, in_sem.at[n_tiles + 5])
    x_cp[0].start()
    for c in wqkv_cp:
        c.start()
    for c in x_cp[1:]:
        c.start()
    wo_cp.start()
    w1_cp.start()
    w2_cp.start()

    sub = lax.broadcasted_iota(jnp.int32, (8, TOK), 0)
    low4 = sub < 4
    ones8 = jnp.ones((8, TOK), F32)
    big8 = jnp.where(sub == 0, BIG, 0.0).astype(F32)

    def norm_tile(i):
        xt = x_v[pl.ds(i * TOK, TOK), :].T
        xt_s[:, pl.ds(i * TOK, TOK)] = xt
        return _layernorm_t(xt.astype(F32)).astype(BF16)

    def head_sq_norms(r):
        sq = [t * t for t in r]
        hi = sq[0] + sq[1] + jnp.where(low4, sq[2], 0.0)
        lo = sq[3] + sq[4] + jnp.where(low4, 0.0, sq[2])
        return jnp.sum(hi, axis=0, keepdims=True), jnp.sum(lo, axis=0, keepdims=True)

    qmax = [None] * N_HEADS
    kmax = [None] * N_HEADS

    def track(store, h, val):
        store[h] = val if store[h] is None else jnp.maximum(store[h], val)

    x_cp[0].wait()
    xn = norm_tile(0)
    for i in range(n_tiles):
        tok = pl.ds(i * TOK, TOK)
        xn_next = None
        for part in range(3):
            if i == 0:
                wqkv_cp[part].wait()
                wqkvt_s[pl.ds(part * dim, dim), :] = wqkv_v[:, pl.ds(part * dim, dim)].T
            if part == 1 and i + 1 < n_tiles:
                x_cp[i + 1].wait()
                xn_next = norm_tile(i + 1)
            for c in range(n_pairs // 2):
                rows = pl.ds(part * dim + c * 2 * pr, 2 * pr)
                y = _dot(wqkvt_s[rows, :], xn)
                blocks = []
                for u in range(2):
                    p = 2 * c + u
                    r = [y[u * pr + 8 * t:u * pr + 8 * t + 8, :] for t in range(5)]
                    if part == 0:
                        r = [t * q_scale for t in r]
                        a, b = head_sq_norms(r)
                        track(qmax, 2 * p, a)
                        track(qmax, 2 * p + 1, b)
                        blk = [r[0] * HI_SCALE, r[1] * HI_SCALE,
                               jnp.where(low4, r[2] * HI_SCALE, 0.0), big8, -big8,
                               jnp.where(low4, 0.0, r[2]), r[3], r[4]]
                        q_s[p, :, tok] = jnp.concatenate(blk, axis=0).astype(BF16)
                    elif part == 1:
                        a, b = head_sq_norms(r)
                        track(kmax, 2 * p, a)
                        track(kmax, 2 * p + 1, b)
                        blocks += [r[0], r[1], r[2], ones8, ones8, r[2], r[3], r[4]]
                    else:
                        r = [t.astype(BF16).astype(F32) for t in r]
                        blk = [r[0], r[1], jnp.where(low4, r[2], 1.0),
                               jnp.where(low4, 1.0, r[2]), r[3], r[4]]
                        v_s[p, :, tok] = jnp.concatenate(blk, axis=0)
                if part == 1:
                    k_s[c, tok, :] = jnp.concatenate(blocks, axis=0).astype(BF16).T
        xn = xn_next

    wo_cp.wait()
    wot_s[...] = wo_v[...].T

    bound = None
    for h in range(N_HEADS):
        b = jnp.max(qmax[h], axis=1, keepdims=True) * jnp.max(kmax[h], axis=1, keepdims=True)
        bound = b if bound is None else jnp.maximum(bound, b)
    limit = (SCORE_BOUND - 1.0) ** 2
    packed_ok = jnp.where(bound <= limit, 1, 0)[0, 0] == 1

    def store_pair(p, tok, acc_hi, acc_lo):
        inv_hi = 1.0 / jnp.broadcast_to(acc_hi[20:21, :], (8, TOK))
        inv_lo = 1.0 / jnp.broadcast_to(acc_lo[0:1, :], (8, TOK))
        o = [acc_hi[0:8] * inv_hi, acc_hi[8:16] * inv_hi,
             jnp.where(low4, acc_hi[16:24] * inv_hi, acc_lo[0:8] * inv_lo),
             acc_lo[8:16] * inv_lo, acc_lo[16:24] * inv_lo]
        ot_s[p, :, tok] = jnp.concatenate(o, axis=0)

    zeros_w = jnp.zeros((64, TOK), BF16)

    @pl.when(packed_ok)
    def _():
        n_blk = seq // KEY_BLK
        groups = n_pairs // PAIRS_PER_STEP

        def step(it, carry):
            tok = pl.ds(pl.multiple_of((it // groups) * TOK, TOK), TOK)
            g = it % groups
            items = [(u, t) for u in range(PAIRS_PER_STEP) for t in range(n_blk)]
            probs = {}
            acc = {}
            for n in range(len(items) + LAG):
                if n < len(items):
                    u, t = items[n]
                    p = g * PAIRS_PER_STEP + u
                    w = q_s[p, :, tok]
                    w = jnp.concatenate([w, zeros_w] if u % 2 == 0 else [zeros_w, w], axis=0)
                    s = _dot(k_s[g * (PAIRS_PER_STEP // 2) + u // 2, pl.ds(t * KEY_BLK, KEY_BLK), :], w)
                    hi = (s + BIG) - BIG
                    probs[n] = (jnp.exp2(s * (1.0 / HI_SCALE)).astype(BF16),
                                jnp.exp2(s - hi).astype(BF16))
                if n >= LAG:
                    u, t = items[n - LAG]
                    p = g * PAIRS_PER_STEP + u
                    pp = probs.pop(n - LAG)
                    for h in range(2):
                        r = _dot(v_s[p, pl.ds(24 * h, 24), pl.ds(t * KEY_BLK, KEY_BLK)], pp[h])
                        acc[h] = r if t == 0 else acc[h] + r
                    if t == n_blk - 1:
                        store_pair(p, tok, acc[0], acc[1])
            return carry

        lax.fori_loop(0, n_tiles * groups, step, 0)

    @pl.when(jnp.logical_not(packed_ok))
    def _():
        row = lax.broadcasted_iota(jnp.int32, (128, TOK), 0)

        def step(it, carry):
            tok = pl.ds(pl.multiple_of((it // n_pairs) * TOK, TOK), TOK)
            p = it % n_pairs
            w = q_s[p, :, tok].astype(F32)
            w = jnp.concatenate([w, w], axis=0)
            base = (p % 2) * 64
            acc = []
            for h in range(2):
                lo_row = base + 40 * h
                keep = (row >= lo_row) & (row < lo_row + 24)
                wh = jnp.where(keep, w, 0.0).astype(BF16)
                s = _dot(k_s[p // 2], wh)
                if h == 0:
                    s = s * (1.0 / HI_SCALE)
                e = jnp.exp2(s - jnp.max(s, axis=0, keepdims=True)).astype(BF16)
                acc.append(_dot(v_s[p, pl.ds(24 * h, 24), :], e))
            store_pair(p, tok, acc[0], acc[1])
            return carry

        lax.fori_loop(0, n_tiles * n_pairs, step, 0)

    w1_cp.wait()
    w2_cp.wait()
    w1t_s[...] = w1_v[...].T
    w2t_s[...] = w2_v[...].T
    ff = w1_v.shape[1]
    b1 = jnp.broadcast_to(b1_ref[...].astype(F32).reshape(1, ff), (128, ff)).T
    b2 = jnp.broadcast_to(b2_ref[...].astype(F32).reshape(1, dim), (128, dim)).T
    b1 = jnp.concatenate([b1] * (TOK // 128), axis=1)
    b2 = jnp.concatenate([b2] * (TOK // 128), axis=1)

    out_cp = [pltpu.make_async_copy(out_v.at[pl.ds(i * TOK, TOK), :],
                                    out_hbm.at[0, pl.ds(i * TOK, TOK), :], out_sem.at[i])
              for i in range(n_tiles)]

    def attn_out(i):
        tok = pl.ds(i * TOK, TOK)
        o = ot_s[:, :, tok].reshape(dim, TOK).astype(BF16)
        h = xt_s[:, tok].astype(F32) + _dot(wot_s[...], o)
        return h, _layernorm_t(h).astype(BF16)

    nxt = attn_out(0)
    for i in range(n_tiles):
        h, hn = nxt
        if i + 1 < n_tiles:
            nxt = attn_out(i + 1)
        a = jnp.maximum(_dot(w1t_s[...], hn) + b1, 0.0)
        a = (a * a).astype(BF16)
        y = h + (_dot(w2t_s[...], a) + b2)
        out_v[pl.ds(i * TOK, TOK), :] = y.astype(BF16).T
        out_cp[i].start()
    for c in out_cp:
        c.wait()


@jax.jit
def pallas_sequential_preLN__softmax_full_mha__dense_activation_squared_relu__prompt_kernel(
    A_x: jax.Array,
    A_wqkv: jax.Array,
    A_wo: jax.Array,
    B_x: jax.Array,
    B_w1: jax.Array,
    B_b1: jax.Array,
    B_w2: jax.Array,
    B_b2: jax.Array,
):
    del B_x
    _, seq, dim = A_x.shape
    ff = B_w1.shape[1]
    dh = dim // N_HEADS
    n_pairs = N_HEADS // 2
    any_spec = pl.BlockSpec(memory_space=pl.ANY)
    vmem_spec = pl.BlockSpec(memory_space=pltpu.VMEM)
    return pl.pallas_call(
        functools.partial(_kernel, seq=seq, dim=dim, dh=dh),
        out_shape=jax.ShapeDtypeStruct(A_x.shape, A_x.dtype),
        in_specs=[any_spec, any_spec, any_spec, any_spec, vmem_spec, any_spec, vmem_spec],
        out_specs=any_spec,
        scratch_shapes=[
            pltpu.VMEM((seq, dim), BF16),
            pltpu.VMEM((dim, 3 * dim), BF16),
            pltpu.VMEM((dim, dim), BF16),
            pltpu.VMEM((dim, ff), BF16),
            pltpu.VMEM((ff, dim), BF16),
            pltpu.VMEM((dim, seq), BF16),
            pltpu.VMEM((3 * dim, dim), BF16),
            pltpu.VMEM((dim, dim), BF16),
            pltpu.VMEM((ff, dim), BF16),
            pltpu.VMEM((dim, ff), BF16),
            pltpu.VMEM((n_pairs // 2, seq, 128), BF16),
            pltpu.VMEM((n_pairs, 64, seq), BF16),
            pltpu.VMEM((n_pairs, 48, seq), F32),
            pltpu.VMEM((n_pairs, 2 * dh, seq), F32),
            pltpu.VMEM((seq, dim), BF16),
            pltpu.SemaphoreType.DMA((seq // TOK + 6,)),
            pltpu.SemaphoreType.DMA((seq // TOK,)),
        ],
        compiler_params=pltpu.CompilerParams(vmem_limit_bytes=110 * 2 ** 20),
        name="fused_block",
    )(A_x, A_wqkv, A_wo, B_w1, B_b1, B_w2, B_b2)
```

```python
import collections
import functools
import math

import jax
import jax.numpy as jnp
from jax import lax
import jax.experimental.pallas as pl
import jax.experimental.pallas.tpu as pltpu

F32 = jnp.float32
BF16 = jnp.bfloat16
I32 = jnp.int32

N_HEADS = 32
LN_EPS = 1e-5
LANES = 128
TOK = 512
ROWS = 64

SCORE_BOUND = 64.0
GRID = 2.0 ** -7
HI_SCALE = 2.0 * SCORE_BOUND / GRID
BIG = 1.5 * 2.0 ** 23 * GRID * HI_SCALE
VALUE_RANGE = 2.0 ** 40

KEY_BLK = 128
SUBS = (48, 16, 32, 32)
LAG = 3
LAG2 = 4
UNITS_PER_STEP = 4
W1_EARLY = 4
WAIT_AT = (0, 4, 18)
WAIT_DELAY = 120
RATES = dict(k0=0.56, q0=0.49, v0=0.48, k1=0.21, q1=0.27, v1=0.43,
             wo0=0.31, wo1=0.72, w10=0.29, w20=0.22, w11=0.55, w21=0.4)
PHASES = dict(q0=1, v1=2, wo1=2, w20=2, w11=2)


def _dot(a, b):
    return lax.dot_general(a, b, (((1,), (0,)), ((), ())), preferred_element_type=F32)


def _blk(i):
    return pl.ds(i * LANES, LANES)


class _SideWork:
    def __init__(self):
        self.urgent = collections.deque()
        self.normal = collections.deque()
        self.credit = self.rate = 0.0
        self.passes = self.phase = 0
        self.anchor = self.anchor_zero = None

    def tune(self, name):
        self.rate, self.phase = RATES[name], PHASES.get(name, 0)

    def add(self, cost, fn, *args):
        self.normal.append((cost, functools.partial(fn, *args)))

    def add_urgent(self, cost, fn, *args):
        self.urgent.append((cost, functools.partial(fn, *args)))

    def anchor_to(self, value=None):
        self.anchor, self.anchor_zero = value, None

    def zero(self):
        if self.anchor is None:
            return 0
        if self.anchor_zero is None:
            n = lax.bitcast_convert_type(self.anchor[0:8, 0:LANES], I32)
            self.anchor_zero = ((n * n + n) & 1)[0, 0] * 256
        return self.anchor_zero

    def rows(self, row0, n):
        if self.anchor is None:
            return pl.ds(row0, n)
        return pl.ds(pl.multiple_of(self.zero() + row0, 16), n)

    def _run(self):
        cost, fn = (self.urgent or self.normal).popleft()
        fn()
        self.credit -= cost

    def tick(self, result):
        self.passes += 1
        if self.passes % 3 == self.phase:
            self.anchor_to(result)
        self.credit = min(self.credit + result.shape[0] * self.rate, 32.0)
        while self.credit > 0 and (self.urgent or self.normal):
            self._run()

    def run_next(self):
        self._run()
        self.credit = max(self.credit, 0.0)

    def flush(self):
        while self.urgent or self.normal:
            self.run_next()


class _Strassen:
    def __init__(self, k_tiles, lhs_refs, side):
        self.lhs, self.side = lhs_refs, side
        self.ready = set()
        self.half, self.odd = k_tiles // 2, k_tiles % 2

    def set_lhs(self, c, k, a11, a12, a21, a22):
        for j, v in enumerate((a11 + a22, a21 + a22, a11, a22, a11 + a12, a21 - a11, a12 - a22)):
            self.lhs[c][j * self.half + k] = v.astype(BF16)
            self.ready.add((c, j * self.half + k))

    def set_lhs_leftover(self, c, top, bot):
        for t, v in enumerate((top, bot)):
            self.lhs[c][7 * self.half + t] = v.astype(BF16)
            self.ready.add((c, 7 * self.half + t))

    @staticmethod
    def rhs_ops(b11, b12, b21, b22):
        return b11 + b22, b11, b12 - b22, b21 - b11, b22, b11 + b12, b21 + b22

    def queue_rhs(self, rhs_ref, ready, x0, x1, cost, before_lane_tile=None):
        h, lanes, add = self.half, range(TOK // LANES), self.side.add

        def combined(k, l, r):
            lo, hi = k * LANES + r, (h + k) * LANES + r
            ops = self.rhs_ops(x0(lo, ROWS, l), x1(lo, ROWS, l), x0(hi, ROWS, l), x1(hi, ROWS, l))
            for j, v in enumerate(ops):
                rhs_ref[j * h + k, l, pl.ds(r, ROWS), :] = v.astype(BF16)

        def leftover(l):
            for t, x in enumerate((x0, x1)):
                rhs_ref[7 * h + t, l] = x(2 * h * LANES, LANES, l).astype(BF16)

        if before_lane_tile is None:
            for k in range(h):
                for l in lanes:
                    for r in range(0, LANES, ROWS):
                        add(cost, combined, k, l, r)
                add(0, ready.update, range(k, 7 * h, h))
            for l in lanes:
                add(cost // 2, leftover, l)
        else:
            for l in lanes:
                before_lane_tile(l)
                for k in range(h):
                    for r in range(0, LANES, ROWS):
                        add(cost, combined, k, l, r)
                add(cost // 2, leftover, l)
        add(0, ready.update, range(7 * h + 2))

    def matmul(self, c, rhs_ref, ready):
        h = self.half

        def one_pass(a, b):
            while (c, a) not in self.ready or b not in ready:
                self.side.run_next()
            rhs = jnp.concatenate([rhs_ref[b, l] for l in range(TOK // LANES)], axis=1)
            y = _dot(self.lhs[c][a], rhs)
            self.side.tick(y)
            return y

        def product(j, acc=None):
            for i in range(j * h, (j + 1) * h):
                y = one_pass(i, i)
                acc = y if acc is None else acc + y
            return acc

        def leftover(half, tile, acc):
            return acc + one_pass(7 * h + half, 7 * h + tile) if self.odd else acc

        m2 = product(1)
        m4 = product(3)
        c21 = leftover(1, 0, m2 + m4)
        m1 = product(0)
        c11 = m1 + m4
        c22 = leftover(1, 1, product(5, m1 - m2))
        m3 = product(2)
        c22 = c22 + m3
        m5 = product(4)
        c11 = c11 - m5
        c12 = leftover(0, 1, m3 + m5)
        c11 = leftover(0, 0, product(6, c11))
        return c11, c12, c21, c22


def _block_kernel(x_hbm, wqkv_hbm, wo_hbm, w1_hbm, b1_hbm, w2_hbm, b2_hbm, out_hbm,
                  x_v, wqkv_v, wo_v, w1_v, w2_v, wt_s, lqkv_s, lo_s, l1_s, l2_s, b1_s, b2_s, xt_s, h_s,
                  rhs_s, hid_s, k_s, q_s, v_s, raw_s, ot_s, out_v, b1_v, b2_v, fence_v, in_sem, out_sem):
    seq, dim = x_v.shape
    ff = w1_v.shape[1]
    dh = dim // N_HEADS
    pr = 2 * dh
    n_tiles, n_pairs, n_lane = seq // TOK, N_HEADS // 2, TOK // LANES
    kd, kf = dim // LANES, ff // LANES
    q_scale = dh ** -0.5 * math.log2(math.e)
    side = _SideWork()

    def rows_of_x(row0, n):
        return x_hbm.at[0, pl.ds(row0, n), :], x_v.at[pl.ds(row0, n), :]

    def cols_of_wqkv(col0, n):
        return wqkv_hbm.at[:, pl.ds(col0, n)], wqkv_v.at[:, pl.ds(col0, n)]

    transfers = dict(
        x0=rows_of_x(0, TOK), x10=rows_of_x(TOK, TOK // 2), x12=rows_of_x(3 * TOK // 2, TOK // 2),
        wk0=cols_of_wqkv(dim, dim - LANES), wk1=cols_of_wqkv(2 * dim - LANES, LANES),
        wq=cols_of_wqkv(0, dim), wv=cols_of_wqkv(2 * dim, dim),
        wo=(wo_hbm, wo_v), x2=rows_of_x(2 * TOK, seq - 2 * TOK), w1=(w1_hbm, w1_v), w2=(w2_hbm, w2_v),
        b1=(b1_hbm, b1_v), b2=(b2_hbm, b2_v), fence=(b1_hbm, fence_v.at[pl.ds(0, ff)]))
    copy = {name: pltpu.make_async_copy(src, dst, in_sem.at[i])
            for i, (name, (src, dst)) in enumerate(transfers.items())}
    for cp in copy.values():
        cp.start()

    def wait(*names):
        for name in names:
            copy[name].wait()

    k_idx = lax.broadcasted_iota(I32, (64, LANES), 0)
    probe = jnp.zeros((64, LANES), F32)
    for k, value in ((0, 60.0), (19, 60.0), (24, BIG), (32, -BIG), (44, 1.5), (63, 1.75)):
        probe = jnp.where(k_idx == k, value, probe)
    probe = _dot(jnp.ones((16, 64), BF16), probe.astype(BF16))[0:1, 0:1]
    wait("x0")

    wqkv, wo, w1 = (_Strassen(kd, refs, side) for refs in (lqkv_s, lo_s, l1_s))
    w2 = _Strassen(kf, l2_s, side)

    sub = lax.broadcasted_iota(I32, (8, TOK), 0)
    low4 = sub < 4
    ones8 = jnp.ones((8, TOK), F32)
    big8 = jnp.where(sub == 0, BIG, 0.0).astype(F32)

    def stage_qkv(part, k, j):
        wt_s[part][k, _blk(j), :] = wqkv_v[side.rows(k * LANES, LANES), _blk(part * kd + j)].astype(F32).T

    def qkv_lhs(part, c, k):
        top, bot = side.rows(4 * pr * c, 2 * pr), side.rows(4 * pr * c + 2 * pr, 2 * pr)
        wt, h = wt_s[part], wqkv.half
        if k == h:
            wqkv.set_lhs_leftover(4 * part + c, wt[2 * h, top, :], wt[2 * h, bot, :])
        else:
            wqkv.set_lhs(4 * part + c, k, wt[k, top, :], wt[h + k, top, :], wt[k, bot, :], wt[h + k, bot, :])

    def queue_qkv_weights(part, chunks):
        for c in chunks:
            for j in ((0, 1), (2,), (3,), (4,))[c]:
                for k in range(kd):
                    side.add(20, stage_qkv, part, k, j)
            for k in range(wqkv.half + 1):
                side.add(45 if k < wqkv.half else 15, qkv_lhs, part, c, k)

    def queue_weights(w, k_tile, chunks):
        def combined(c, k):
            a, b = k_tile(k, c).astype(F32).T, k_tile(w.half + k, c).astype(F32).T
            w.set_lhs(c, k, a[:ROWS], b[:ROWS], a[ROWS:], b[ROWS:])

        def leftover(c):
            a = k_tile(2 * w.half, c).astype(F32).T
            w.set_lhs_leftover(c, a[:ROWS], a[ROWS:])

        for c in chunks:
            for k in range(w.half):
                side.add(55, combined, c, k)
            if w.odd:
                side.add(20, leftover, c)

    def k_tile_of(w_ref):
        return lambda k, c: w_ref[side.rows(k * LANES, LANES), _blk(c)]

    def w2_k_tile(k, c):
        row0 = (k % w2.half) * 2 * LANES + (k // w2.half) * ROWS
        return jnp.concatenate([w2_v[side.rows(row0 + d, ROWS), _blk(c)].astype(F32) for d in (0, LANES)], axis=0)

    def bias_column(b_ref, b_s):
        n = b_ref.shape[0]
        b_s[...] = jnp.broadcast_to(b_ref[...].astype(F32).reshape(1, n), (LANES, n)).T

    stats = {}

    def accumulate(key, rows):
        if key not in stats:
            stats[key] = (rows[0:1], None, None)
        shift, s1, s2 = stats[key]
        d = (rows - shift).reshape(rows.shape[0] // 8, 8, rows.shape[1])
        t1, t2 = jnp.sum(d, axis=0), jnp.sum(d * d, axis=0)
        stats[key] = (shift, t1 if s1 is None else s1 + t1, t2 if s2 is None else s2 + t2)

    def moments(key):
        shift, s1, s2 = stats.pop(key)
        m = jnp.sum(s1, axis=0, keepdims=True) * (1.0 / dim)
        v = jnp.sum(s2, axis=0, keepdims=True) * (1.0 / dim) - m * m
        stats[key] = (shift + m, lax.rsqrt(jnp.maximum(v, 0.0) + LN_EPS))

    def normalized(source, stat):
        def load(row, n, l):
            mean, rstd = stat(l)
            return (source(side.rows(row, n), l) - mean) * rstd
        return load

    def transpose_x(i, l, k):
        xt = x_v[side.rows(i * TOK + l * LANES, LANES), _blk(k)].astype(F32).T
        xt_s[i][l][_blk(k), :] = xt
        accumulate(("x", i, l), xt)

    def queue_transpose(i, l):
        for k in range(kd):
            side.add(30, transpose_x, i, l, k)
        side.add(0, moments, ("x", i, l))

    def queue_input(s, before_lane_tile=None):
        x0, x1 = [normalized(lambda rows, l, i=i: xt_s[i][l][rows, :], lambda l, i=i: stats["x", i, l])
                  for i in (2 * s, 2 * s + 1)]
        wqkv.queue_rhs(rhs_s[s], ready_qkv[s], x0, x1, 34, before_lane_tile)

    peak = {}

    def track(key, value):
        peak[key] = jnp.maximum(peak[key], value) if key in peak else value

    def track_norms(name, p, r):
        sq = [t * t for t in r]
        first = sq[0] + sq[1] + jnp.where(low4, sq[2], 0.0)
        second = sq[3] + sq[4] + jnp.where(low4, 0.0, sq[2])
        for h, value in ((2 * p, first), (2 * p + 1, second)):
            track((name, h), jnp.sum(value, axis=0, keepdims=True))

    def pair_rows(y):
        return [y[8 * t:8 * t + 8, :] for t in range(5)]

    def emit_q(y, p, i):
        r = [t * q_scale for t in pair_rows(y)]
        track_norms("q", p, r)
        rows = [r[0] * HI_SCALE, r[1] * HI_SCALE, jnp.where(low4, r[2] * HI_SCALE, 0.0),
                big8, -big8, jnp.where(low4, 0.0, r[2]), r[3], r[4]]
        q_s[i, p] = jnp.concatenate(rows, axis=0).astype(BF16)

    def emit_k(y, p, i):
        rows = []
        for u in range(2):
            r = pair_rows(y[u * pr:(u + 1) * pr])
            track_norms("k", p + u, r)
            rows += [r[0], r[1], r[2], ones8, ones8, r[2], r[3], r[4]]
        k_s[p // 2, pl.ds(i * TOK, TOK), :] = jnp.concatenate(rows, axis=0).T.astype(BF16)

    def emit_v(y, p, i):
        r = [t.astype(BF16).astype(F32) for t in pair_rows(y)]
        rows = [r[0], r[1], jnp.where(low4, r[2], 1.0), jnp.where(low4, 1.0, r[2]), r[3], r[4]]
        v_s[p, :, pl.ds(i * TOK, TOK)] = jnp.concatenate(rows, axis=0)
        size = functools.reduce(jnp.maximum, [jnp.abs(t) for t in r])
        track("v", functools.reduce(jnp.maximum, [size[:, l * LANES:(l + 1) * LANES] for l in range(n_lane)]))

    def score_bound():
        sq = [jnp.max(jnp.concatenate([peak[name, h] for h in range(N_HEADS)], axis=0), axis=1, keepdims=True)
              for name in "qk"]
        peak["score^2"] = jnp.max(sq[0] * sq[1], axis=0, keepdims=True)

    ready_qkv, ready_wo, ready_w1, ready_w2 = ([set(), set()] for _ in range(4))
    for l in range(n_lane):
        queue_transpose(0, l)
    side.add(0, lambda: side.anchor_to(x_v[0:16, 0:LANES].astype(F32)))

    def arriving(l):
        if l % 2 == 0:
            side.add(0, wait, "x1%d" % l)
        queue_transpose(1, l)

    queue_input(0, arriving)
    side.add(0, wait, "wk0")
    side.add(0, side.anchor_to)
    queue_qkv_weights(1, range(3))
    side.flush()

    def after_step(n):
        if n == WAIT_AT[0]:
            side.add(WAIT_DELAY, lambda: None)
            side.add(0, wait, "wk1", "wq")
            queue_qkv_weights(1, range(3, 4))
            queue_qkv_weights(0, range(4))
        if n == WAIT_AT[1]:
            side.add(WAIT_DELAY, lambda: None)
            side.add(0, wait, "wv", "wo", "x2")
            queue_qkv_weights(2, range(4))
            for i in (2, 3):
                for l in range(n_lane):
                    queue_transpose(i, l)
            queue_input(1)
        if n == WAIT_AT[2]:
            queue_weights(wo, k_tile_of(wo_v), range(kd))

    for s in range(2):
        for n, part in enumerate((1, 0, 2)):
            side.tune("qkv"[part] + str(s))
            for c in range(4):
                c11, c12, c21, c22 = wqkv.matmul(4 * part + c, rhs_s[s], ready_qkv[s])
                for y, p, i in ((c21, 4 * c + 2, 2 * s), (c22, 4 * c + 2, 2 * s + 1),
                                (c12, 4 * c, 2 * s + 1), (c11, 4 * c, 2 * s)):
                    if part == 1:
                        side.add_urgent(64, emit_k, y, p, i)
                    else:
                        for u in range(2):
                            side.add_urgent(28, emit_v if part else emit_q, y[u * pr:(u + 1) * pr], p + u, i)
                after_step(12 * s + 4 * n + c)
            if (n, s) == (1, 1):
                side.add_urgent(150, score_bound)
    side.flush()
    wait("w1", "w2", "b1", "b2")
    v_size = jnp.max(jnp.max(peak["v"], axis=1, keepdims=True), axis=0, keepdims=True)
    safe = ((peak["score^2"] <= (SCORE_BOUND - 1.0) ** 2) & (probe == GRID * HI_SCALE + 3.25)
            & (v_size <= VALUE_RANGE) & (v_size >= 1.0 / VALUE_RANGE))
    packed = jnp.where(safe, 1, 0)[0, 0] == 1

    n_units = n_tiles * n_pairs

    def store_pair(p, i, first, second):
        inv = 1.0 / jnp.where(low4, second[0:8], first[16:24])
        swapped = jnp.concatenate([inv[4:8], inv[0:4]], axis=0)
        inv1, inv2 = jnp.where(low4, swapped, inv), jnp.where(low4, inv, swapped)
        ot_s[i, p] = jnp.concatenate(
            [first[0:8] * inv1, first[8:16] * inv1, jnp.where(low4, first[16:24] * inv1, second[0:8] * inv2),
             second[8:16] * inv2, second[16:24] * inv2], axis=0)

    def store_raw(unit):
        store_pair(unit % n_pairs, unit // n_pairs, raw_s[0], raw_s[1])

    @pl.when(packed)
    def _():
        n_blk = seq // KEY_BLK
        items = [(u, t) for u in range(UNITS_PER_STEP) for t in range(n_blk)]
        raw_s[...] = jnp.ones(raw_s.shape, F32)

        def step(it, carry):
            unit0 = it * UNITS_PER_STEP
            store_raw(jnp.maximum(unit0 - 1, 0))

            def locate(u):
                return (unit0 + u) // n_pairs, (unit0 + u) % n_pairs

            scores, probs, acc = {}, {}, {}
            for n in range(len(items) + max(LAG, LAG2)):
                if n < len(items):
                    u, t = items[n]
                    i, p = locate(u)
                    scores[n] = jnp.concatenate(
                        [_dot(k_s[p // 2, pl.ds(t * KEY_BLK + sum(SUBS[:j]), r), pl.ds(64 * (u % 2), 64)], q_s[i, p])
                         for j, r in enumerate(SUBS)], axis=0)
                if 1 <= n <= len(items):
                    s = scores.pop(n - 1)
                    first = jnp.exp2(s * (1.0 / HI_SCALE)).astype(BF16)
                    second = jnp.exp2(s - ((s + BIG) - BIG)).astype(BF16)
                    probs[n - 1] = (first, second)
                for h in (1, 0):
                    m = n - (LAG, LAG2)[h]
                    if 0 <= m < len(items):
                        u, t = items[m]
                        i, p = locate(u)
                        r = _dot(v_s[p, pl.ds(24 * h, 24), pl.ds(t * KEY_BLK, KEY_BLK)], probs[m][h])
                        acc[u, h] = r if t == 0 else acc[u, h] + r
                        if t == n_blk - 1 and u == UNITS_PER_STEP - 1:
                            raw_s[h] = acc[u, h]
                m = n - max(LAG, LAG2)
                if 0 <= m < len(items) and items[m][1] == n_blk - 1 and items[m][0] < UNITS_PER_STEP - 1:
                    u = items[m][0]
                    i, p = locate(u)
                    store_pair(p, i, acc[u, 0], acc[u, 1])
            return carry

        lax.fori_loop(0, n_units // UNITS_PER_STEP, step, 0)

    @pl.when(jnp.logical_not(packed))
    def _():
        row = lax.broadcasted_iota(I32, (128, TOK), 0)

        def head(it, carry):
            unit, h = it // 2, it % 2
            i, p = unit // n_pairs, unit % n_pairs
            w = q_s[i, p].astype(F32)
            row0 = (p % 2) * 64 + 40 * h
            w = jnp.where((row >= row0) & (row < row0 + 24), jnp.concatenate([w, w], axis=0), 0.0)
            s = _dot(k_s[p // 2], w.astype(BF16)) * jnp.where(h == 0, 1.0 / HI_SCALE, 1.0)
            e = jnp.exp2(s - jnp.max(s, axis=0, keepdims=True)).astype(BF16)
            raw_s[h] = _dot(v_s[p, pl.ds(pl.multiple_of(24 * h, 8), 24), :], e)

            @pl.when(h == 1)
            def _():
                store_raw(unit)

            return carry

        lax.fori_loop(0, 2 * n_units, head, 0)

    side.anchor_to()
    store_raw(n_units - 1)

    def attn_rows(i, row, n, l):
        return jnp.concatenate([ot_s[side.zero() + i, r // pr, pl.ds(r % pr, 8), _blk(l)]
                                for r in range(row, row + n, 8)], axis=0)

    def add_residual(i, row0, y):
        rows = pl.ds(row0, ROWS)
        h = jnp.concatenate([xt[rows, :] for xt in xt_s[i]], axis=1) + y
        h_s[i][rows, :] = h
        accumulate(("h", i), h)

    def activate(s, c, l, y):
        a = []
        for j in range(4):
            bias = b1_s[pl.ds(c * LANES + (j // 2) * ROWS, ROWS), :]
            t = jnp.maximum(y[j][:, l * LANES:(l + 1) * LANES] + bias, 0.0)
            a.append(t * t)
        for j, v in enumerate(w2.rhs_ops(*a)):
            hid_s[s][j * w2.half + c // 2, l, pl.ds(c % 2 * ROWS, ROWS), :] = v.astype(BF16)

    def finish(i, c, top, bot):
        y = jnp.concatenate([top, bot], axis=0) + jnp.concatenate([b2_s[_blk(c), :]] * n_lane, axis=1)
        out_v[pl.ds(i * TOK, TOK), _blk(c)] = (h_s[i][_blk(c), :] + y).T.astype(BF16)

    parts = ((pl.ds(0, 2 * TOK), pl.ds(0, dim)), (pl.ds(2 * TOK, 2 * TOK), pl.ds(0, dim - LANES)),
             (pl.ds(2 * TOK, 2 * TOK), _blk(kd - 1)))
    out_cp = [pltpu.make_async_copy(out_v.at[rows, cols], out_hbm.at[0, rows, cols], out_sem.at[j])
              for j, (rows, cols) in enumerate(parts)]

    def send(cp, earlier):
        cp.start()
        earlier.wait()

    for s in range(2):
        x0, x1 = [functools.partial(attn_rows, i) for i in (2 * s, 2 * s + 1)]
        wo.queue_rhs(rhs_s[2 + s], ready_wo[s], x0, x1, 28)
    side.add(200, bias_column, b1_v, b1_s)
    queue_weights(w1, k_tile_of(w1_v), range(W1_EARLY))
    for s in range(2):
        side.tune("wo%d" % s)
        for c in range(kd):
            c11, c12, c21, c22 = wo.matmul(c, rhs_s[2 + s], ready_wo[s])
            for y, i, r0 in ((c21, 2 * s, ROWS), (c22, 2 * s + 1, ROWS), (c12, 2 * s + 1, 0), (c11, 2 * s, 0)):
                side.add_urgent(50, add_residual, i, c * LANES + r0, y)
        for i in (2 * s, 2 * s + 1):
            side.add_urgent(10, moments, ("h", i))
        x0, x1 = [normalized(lambda rows, l, i=i: h_s[i][rows, _blk(l)],
                             lambda l, i=i: [t[:, l * LANES:(l + 1) * LANES] for t in stats["h", i]])
                  for i in (2 * s, 2 * s + 1)]
        w1.queue_rhs(rhs_s[s], ready_w1[s], x0, x1, 34)
        if s == 0:
            queue_weights(w1, k_tile_of(w1_v), range(W1_EARLY, kf))
        else:
            side.add(80, bias_column, b2_v, b2_s)
            queue_weights(w2, w2_k_tile, range(kd))
    for s in range(2):
        side.tune("w1%d" % s)
        for c in range(kf):
            y = w1.matmul(c, rhs_s[s], ready_w1[s])
            for l in range(n_lane):
                side.add_urgent(42, activate, s, c, l, y)
            if c % 2:
                side.add_urgent(0, ready_w2[s].update, range(c // 2, 7 * w2.half, w2.half))
        side.tune("w2%d" % s)
        for c in range(kd):
            c11, c12, c21, c22 = w2.matmul(c, hid_s[s], ready_w2[s])
            side.add_urgent(70, finish, 2 * s + 1, c, c12, c22)
            side.add_urgent(70, finish, 2 * s, c, c11, c21)
            if (s, c) in ((1, 0), (1, kd - 2)):
                side.add_urgent(100, lambda: None)
                side.add_urgent(0, send, *((out_cp[0], copy["fence"]) if c == 0 else (out_cp[1], out_cp[0])))
    side.flush()
    out_cp[2].start()
    out_cp[1].wait()
    out_cp[2].wait()


@jax.jit
def pallas_sequential_preLN__softmax_full_mha__dense_activation_squared_relu__prompt_kernel(
    A_x: jax.Array,
    A_wqkv: jax.Array,
    A_wo: jax.Array,
    B_x: jax.Array,
    B_w1: jax.Array,
    B_b1: jax.Array,
    B_w2: jax.Array,
    B_b2: jax.Array,
):
    del B_x
    _, seq, dim = A_x.shape
    ff = B_w1.shape[1]
    assert (seq, dim, ff) == (4 * TOK, 20 * N_HEADS, 12 * LANES), "the tiling is laid out for these shapes"
    n_pairs, n_tiles, n_lane = N_HEADS // 2, seq // TOK, TOK // LANES
    pr = 2 * dim // N_HEADS
    kd, kf = dim // LANES, ff // LANES
    ops_d, ops_f = 7 * (kd // 2) + 2, 7 * (kf // 2)
    any_spec = pl.BlockSpec(memory_space=pl.ANY)
    return pl.pallas_call(
        _block_kernel,
        out_shape=jax.ShapeDtypeStruct(A_x.shape, A_x.dtype),
        in_specs=[any_spec] * 7,
        out_specs=any_spec,
        scratch_shapes=[
            pltpu.VMEM((seq, dim), BF16),
            pltpu.VMEM((dim, 3 * dim), BF16),
            pltpu.VMEM((dim, dim), BF16),
            pltpu.VMEM((dim, ff), BF16),
            pltpu.VMEM((ff, dim), BF16),
            [pltpu.VMEM((kd, dim, LANES), F32)] * 3,
            [pltpu.VMEM((ops_d, 2 * pr, LANES), BF16)] * (3 * n_pairs // 4),
            [pltpu.VMEM((ops_d, ROWS, LANES), BF16)] * kd,
            [pltpu.VMEM((ops_d, ROWS, LANES), BF16)] * kf,
            [pltpu.VMEM((ops_f, ROWS, LANES), BF16)] * kd,
            pltpu.VMEM((ff, LANES), F32),
            pltpu.VMEM((dim, LANES), F32),
            [[pltpu.VMEM((dim, LANES), F32)] * n_lane] * n_tiles,
            [pltpu.VMEM((dim, TOK), F32)] * n_tiles,
            [pltpu.VMEM((ops_d, n_lane, LANES, LANES), BF16)] * 4,
            [pltpu.VMEM((ops_f, n_lane, LANES, LANES), BF16)] * 2,
            pltpu.VMEM((n_pairs // 2, seq, LANES), BF16),
            pltpu.VMEM((n_tiles, n_pairs, 64, TOK), BF16),
            pltpu.VMEM((n_pairs, 48, seq), F32),
            pltpu.VMEM((2, 24, TOK), F32),
            pltpu.VMEM((n_tiles, n_pairs, pr, TOK), F32),
            pltpu.VMEM((seq, dim), BF16),
            pltpu.VMEM((ff,), BF16),
            pltpu.VMEM((dim,), BF16),
            pltpu.VMEM((23 * 256,), BF16),
            pltpu.SemaphoreType.DMA((14,)),
            pltpu.SemaphoreType.DMA((3,)),
        ],
        compiler_params=pltpu.CompilerParams(vmem_limit_bytes=110 * 2 ** 20),
        name="fused_block",
    )(A_x, A_wqkv, A_wo, B_w1, B_b1, B_w2, B_b2)
```

```python
import collections
import functools
import math

import jax
import jax.numpy as jnp
from jax import lax
import jax.experimental.pallas as pl
import jax.experimental.pallas.tpu as pltpu

F32 = jnp.float32
BF16 = jnp.bfloat16
I32 = jnp.int32

N_HEADS = 32
LN_EPS = 1e-5
LANES = 128
TOK = 512
ROWS = 64

SCORE_BOUND = 64.0
GRID = 2.0 ** -7
HI_SCALE = 2.0 * SCORE_BOUND / GRID
BIG = 1.5 * 2.0 ** 23 * GRID * HI_SCALE
WEIGHT_RANGE = 2.0 ** 30

KEY_BLK = 128
SUBS = (64, 32, 32)
LAGS = (3, 4)
LOOPS = ((0, 1, 4), (4, 10, 6))
W1_EARLY = 4
WAIT_AT = (1, 3, 13)
WAIT_DELAY = 120
MAX_CREDIT = 32
RATES = dict(k0=0.45, q0=0.6, v0=0.32, k1=0.17, q1=0.1, v1=0.55,
             wo0=0.31, wo1=0.79, w10=0.29, w20=0.33, w11=0.24, w21=0.4)
PHASES = dict(q0=4, k0=4, v0=1, q1=1, k1=4, v1=2, wo0=3, wo1=2, w10=3, w20=5, w11=1)
PERIODS = dict(v0=5, k0=6, q1=9, k1=4, v1=6, w10=9, wo1=5, wo0=9)


def _dot(a, b):
    return lax.dot_general(a, b, (((1,), (0,)), ((), ())), preferred_element_type=F32)


def _first_score(s):
    return s * (1.0 / HI_SCALE)


def _second_score(s):
    return s - ((s + BIG) - BIG)


def _blk(i):
    return pl.ds(i * LANES, LANES)


class _SideWork:
    def __init__(self):
        self.urgent = collections.deque()
        self.normal = collections.deque()
        self.credit = self.rate = 0.0
        self.passes = self.phase = 0
        self.period = 3
        self.anchor = self.anchor_zero = None

    def tune(self, name):
        self.rate, self.phase, self.period = RATES[name], PHASES.get(name, 0), PERIODS.get(name, 3)

    def add(self, cost, fn, *args):
        self.normal.append((cost, functools.partial(fn, *args)))

    def add_urgent(self, cost, fn, *args):
        self.urgent.append((cost, functools.partial(fn, *args)))

    def anchor_to(self, value=None):
        self.anchor, self.anchor_zero = value, None

    def zero(self):
        if self.anchor is None:
            return 0
        if self.anchor_zero is None:
            n = lax.bitcast_convert_type(self.anchor[0:8, 0:LANES], I32)
            self.anchor_zero = ((n * n + n) & 1)[0, 0] * 256
        return self.anchor_zero

    def rows(self, row0, n):
        if self.anchor is None:
            return pl.ds(row0, n)
        return pl.ds(pl.multiple_of(self.zero() + row0, 16), n)

    def _run(self):
        cost, fn = (self.urgent or self.normal).popleft()
        fn()
        self.credit -= cost

    def tick(self, result):
        self.passes += 1
        if self.passes % self.period == self.phase % self.period:
            self.anchor_to(result)
        self.credit = min(self.credit + result.shape[0] * self.rate, MAX_CREDIT)
        while self.credit > 0 and (self.urgent or self.normal):
            self._run()

    def run_next(self):
        self._run()
        self.credit = max(self.credit, 0.0)

    def flush(self):
        while self.urgent or self.normal:
            self.run_next()


class _Strassen:
    def __init__(self, k_tiles, lhs_refs, side):
        self.lhs, self.side = lhs_refs, side
        self.ready = set()
        self.half, self.odd = k_tiles // 2, k_tiles % 2

    def set_lhs(self, c, k, a11, a12, a21, a22):
        for j, v in enumerate((a11 + a22, a21 + a22, a11, a22, a11 + a12, a21 - a11, a12 - a22)):
            self.lhs[c][j * self.half + k] = v.astype(BF16)
            self.ready.add((c, j * self.half + k))

    def set_lhs_leftover(self, c, top, bot):
        for t, v in enumerate((top, bot)):
            self.lhs[c][7 * self.half + t] = v.astype(BF16)
            self.ready.add((c, 7 * self.half + t))

    @staticmethod
    def rhs_ops(b11, b12, b21, b22):
        return b11 + b22, b11, b12 - b22, b21 - b11, b22, b11 + b12, b21 + b22

    def queue_rhs(self, rhs_ref, ready, x0, x1, cost, before_lane_tile=None):
        h, lanes, add = self.half, range(TOK // LANES), self.side.add

        def combined(k, l, r):
            lo, hi = k * LANES + r, (h + k) * LANES + r
            ops = self.rhs_ops(x0(lo, ROWS, l), x1(lo, ROWS, l), x0(hi, ROWS, l), x1(hi, ROWS, l))
            for j, v in enumerate(ops):
                rhs_ref[j * h + k, l, pl.ds(r, ROWS), :] = v.astype(BF16)

        def leftover(l):
            for t, x in enumerate((x0, x1)):
                rhs_ref[7 * h + t, l] = x(2 * h * LANES, LANES, l).astype(BF16)

        if before_lane_tile is None:
            for k in range(h):
                for l in lanes:
                    for r in range(0, LANES, ROWS):
                        add(cost, combined, k, l, r)
                add(0, ready.update, range(k, 7 * h, h))
            for l in lanes:
                add(cost // 2, leftover, l)
        else:
            for l in lanes:
                before_lane_tile(l)
                for k in range(h):
                    for r in range(0, LANES, ROWS):
                        add(cost, combined, k, l, r)
                add(cost // 2, leftover, l)
        add(0, ready.update, range(7 * h + 2))

    def matmul(self, c, rhs_ref, ready, done):
        h = self.half

        def one_pass(a, b):
            while (c, a) not in self.ready or b not in ready:
                self.side.run_next()
            rhs = jnp.concatenate([rhs_ref[b, l] for l in range(TOK // LANES)], axis=1)
            y = _dot(self.lhs[c][a], rhs)
            self.side.tick(y)
            return y

        def product(j, acc=None):
            for i in range(j * h, (j + 1) * h):
                y = one_pass(i, i)
                acc = y if acc is None else acc + y
            return acc

        def leftover(half, tile, acc):
            return acc + one_pass(7 * h + half, 7 * h + tile) if self.odd else acc

        m2 = product(1)
        m4 = product(3)
        done(1, 0, leftover(1, 0, m2 + m4))
        m1 = product(0)
        c11 = m1 + m4
        c22 = leftover(1, 1, product(5, m1 - m2))
        m3 = product(2)
        done(1, 1, c22 + m3)
        m5 = product(4)
        c11 = c11 - m5
        done(0, 1, leftover(0, 1, m3 + m5))
        done(0, 0, leftover(0, 0, product(6, c11)))


def _block_kernel(x_hbm, wqkv_hbm, wo_hbm, w1_hbm, b1_hbm, w2_hbm, b2_hbm, out_hbm,
                  x_v, wqkv_v, wo_v, w1_v, w2_v, wt_s, lqkv_s, lo_s, l1_s, l2_s, b1_s, b2_s, xt_s, h_s,
                  rhs_s, hid_s, k_s, q_s, v_s, raw_s, ot_s, out_v, b1_v, b2_v, fence_v, in_sem, out_sem):
    seq, dim = x_v.shape
    ff = w1_v.shape[1]
    dh = dim // N_HEADS
    pr = 2 * dh
    n_tiles, n_pairs, n_lane = seq // TOK, N_HEADS // 2, TOK // LANES
    kd, kf = dim // LANES, ff // LANES
    q_scale = dh ** -0.5 * math.log2(math.e)
    side = _SideWork()

    def rows_of_x(row0, n):
        return x_hbm.at[0, pl.ds(row0, n), :], x_v.at[pl.ds(row0, n), :]

    def cols_of_wqkv(col0, n):
        return wqkv_hbm.at[:, pl.ds(col0, n)], wqkv_v.at[:, pl.ds(col0, n)]

    transfers = dict(
        x0=rows_of_x(0, TOK), x10=rows_of_x(TOK, TOK // 2), x12=rows_of_x(3 * TOK // 2, TOK // 2),
        wk0=cols_of_wqkv(dim, dim - LANES), wk1=cols_of_wqkv(2 * dim - LANES, LANES),
        wq=cols_of_wqkv(0, dim), wv=cols_of_wqkv(2 * dim, dim),
        wo=(wo_hbm, wo_v), x2=rows_of_x(2 * TOK, seq - 2 * TOK), w1=(w1_hbm, w1_v), w2=(w2_hbm, w2_v),
        b1=(b1_hbm, b1_v), b2=(b2_hbm, b2_v), fence=(b1_hbm, fence_v.at[pl.ds(0, ff)]))
    copy = {name: pltpu.make_async_copy(src, dst, in_sem.at[i])
            for i, (name, (src, dst)) in enumerate(transfers.items())}
    for cp in copy.values():
        cp.start()

    def wait(*names):
        for name in names:
            copy[name].wait()

    k_idx = lax.broadcasted_iota(I32, (64, LANES), 0)
    probe = jnp.zeros((64, LANES), F32)
    for k, value in ((0, 60.0), (19, 60.0), (24, BIG), (32, -BIG), (44, 1.5), (63, 1.75)):
        probe = jnp.where(k_idx == k, value, probe)
    probe = _dot(jnp.ones((16, 64), BF16), probe.astype(BF16))[0:1, 0:1]
    probe_ok = (probe == GRID * HI_SCALE + 3.25) & (_second_score(probe) == 3.25)
    wait("x0")

    wqkv, wo, w1 = (_Strassen(kd, refs, side) for refs in (lqkv_s, lo_s, l1_s))
    w2 = _Strassen(kf, l2_s, side)

    sub = lax.broadcasted_iota(I32, (8, TOK), 0)
    low4 = sub < 4
    ones8 = jnp.ones((8, TOK), F32)
    big8 = jnp.where(sub == 0, BIG, 0.0).astype(F32)

    peak = {}

    def track(key, value):
        peak[key] = jnp.maximum(peak[key], value) if key in peak else value

    def stage_qkv(part, k, j):
        w = wqkv_v[side.rows(k * LANES, LANES), _blk(part * kd + j)].astype(F32)
        wt_s[part][k, _blk(j), :] = w.T
        if part == 2:
            track("wv", jnp.max(jnp.abs(w).reshape(LANES // 8, 8, LANES), axis=0))

    def qkv_lhs(part, c, k):
        top, bot = side.rows(4 * pr * c, 2 * pr), side.rows(4 * pr * c + 2 * pr, 2 * pr)
        wt, h = wt_s[part], wqkv.half
        if k == h:
            wqkv.set_lhs_leftover(4 * part + c, wt[2 * h, top, :], wt[2 * h, bot, :])
        else:
            wqkv.set_lhs(4 * part + c, k, wt[k, top, :], wt[h + k, top, :], wt[k, bot, :], wt[h + k, bot, :])

    def queue_qkv_weights(part, chunks):
        for c in chunks:
            for j in ((0, 1), (2,), (3,), (4,))[c]:
                for k in range(kd):
                    side.add(20, stage_qkv, part, k, j)
            for k in range(wqkv.half + 1):
                side.add(45 if k < wqkv.half else 15, qkv_lhs, part, c, k)

    def queue_weights(w, k_tile, chunks):
        def combined(c, k):
            a, b = k_tile(k, c).astype(F32).T, k_tile(w.half + k, c).astype(F32).T
            w.set_lhs(c, k, a[:ROWS], b[:ROWS], a[ROWS:], b[ROWS:])

        def leftover(c):
            a = k_tile(2 * w.half, c).astype(F32).T
            w.set_lhs_leftover(c, a[:ROWS], a[ROWS:])

        for c in chunks:
            for k in range(w.half):
                side.add(55, combined, c, k)
            if w.odd:
                side.add(20, leftover, c)

    def k_tile_of(w_ref):
        return lambda k, c: w_ref[side.rows(k * LANES, LANES), _blk(c)]

    def w2_k_tile(k, c):
        row0 = (k % w2.half) * 2 * LANES + (k // w2.half) * ROWS
        return jnp.concatenate([w2_v[side.rows(row0 + d, ROWS), _blk(c)].astype(F32) for d in (0, LANES)], axis=0)

    def bias_column(b_ref, b_s):
        n = b_ref.shape[0]
        b_s[...] = jnp.broadcast_to(b_ref[...].astype(F32).reshape(1, n), (LANES, n)).T

    stats = {}

    def accumulate(key, rows):
        if key not in stats:
            stats[key] = (rows[0:1], None, None)
        shift, s1, s2 = stats[key]
        d = (rows - shift).reshape(rows.shape[0] // 8, 8, rows.shape[1])
        t1, t2 = jnp.sum(d, axis=0), jnp.sum(d * d, axis=0)
        stats[key] = (shift, t1 if s1 is None else s1 + t1, t2 if s2 is None else s2 + t2)

    def moments(key):
        shift, s1, s2 = stats.pop(key)
        m = jnp.sum(s1, axis=0, keepdims=True) * (1.0 / dim)
        v = jnp.sum(s2, axis=0, keepdims=True) * (1.0 / dim) - m * m
        stats[key] = (shift + m, lax.rsqrt(jnp.maximum(v, 0.0) + LN_EPS))

    def normalized(source, stat):
        def load(row, n, l):
            mean, rstd = stat(l)
            return (source(side.rows(row, n), l) - mean) * rstd
        return load

    def transpose_x(i, l, k):
        xt = x_v[side.rows(i * TOK + l * LANES, LANES), _blk(k)].astype(F32).T
        xt_s[i][l][_blk(k), :] = xt
        accumulate(("x", i, l), xt)

    def queue_transpose(i, l):
        for k in range(kd):
            side.add(30, transpose_x, i, l, k)
        side.add(0, moments, ("x", i, l))

    def queue_input(s, before_lane_tile=None):
        x0, x1 = [normalized(lambda rows, l, i=i: xt_s[i][l][rows, :], lambda l, i=i: stats["x", i, l])
                  for i in (2 * s, 2 * s + 1)]
        wqkv.queue_rhs(rhs_s[s], ready_qkv[s], x0, x1, 34, before_lane_tile)

    def track_norms(name, p, r):
        sq = [t * t for t in r]
        first = sq[0] + sq[1] + jnp.where(low4, sq[2], 0.0)
        second = sq[3] + sq[4] + jnp.where(low4, 0.0, sq[2])
        for h, value in ((2 * p, first), (2 * p + 1, second)):
            track((name, h), jnp.sum(value, axis=0, keepdims=True))

    def pair_rows(y):
        return [y[8 * t:8 * t + 8, :] for t in range(5)]

    def emit_q(y, p, i):
        r, first = pair_rows(y), q_scale * HI_SCALE
        track_norms("q", p, r)
        rows = [r[0] * first, r[1] * first, jnp.where(low4, r[2] * first, 0.0), big8, -big8,
                jnp.where(low4, 0.0, r[2] * q_scale), r[3] * q_scale, r[4] * q_scale]
        q_s[i, p] = jnp.concatenate(rows, axis=0).astype(BF16)

    def emit_k(y, p, i):
        rows = []
        for u in range(2):
            r = pair_rows(y[u * pr:(u + 1) * pr])
            track_norms("k", p + u, r)
            rows += [r[0], r[1], r[2], ones8, ones8, r[2], r[3], r[4]]
        k_s[p // 2, pl.ds(i * TOK, TOK), :] = jnp.concatenate(rows, axis=0).T.astype(BF16)

    def emit_v(y, p, i):
        r = [t.astype(BF16).astype(F32) for t in pair_rows(y)]
        rows = [r[0], r[1], jnp.where(low4, r[2], 1.0), jnp.where(low4, 1.0, r[2]), r[3], r[4]]
        v_s[p, :, pl.ds(i * TOK, TOK)] = jnp.concatenate(rows, axis=0)

    def emit(part, s, c, half, tile, y):
        p, i = 4 * c + 2 * half, 2 * s + tile
        if part == 1:
            side.add_urgent(64, emit_k, y, p, i)
        else:
            for u in range(2):
                side.add_urgent(28, emit_v if part else emit_q, y[u * pr:(u + 1) * pr], p + u, i)

    packed = []

    def range_check():
        sq = [jnp.max(jnp.concatenate([peak[name, h] for h in range(N_HEADS)], axis=0), axis=1, keepdims=True)
              for name in "qk"]
        score_sq = jnp.max(sq[0] * sq[1], axis=0, keepdims=True)
        wv = jnp.max(jnp.max(peak["wv"], axis=1, keepdims=True), axis=0, keepdims=True)
        safe = ((score_sq <= ((SCORE_BOUND - 1.0) / q_scale) ** 2) & probe_ok
                & (wv <= WEIGHT_RANGE) & (wv >= 1.0 / WEIGHT_RANGE))
        packed.append(jnp.where(safe, 1, 0)[0, 0])

    ready_qkv, ready_wo, ready_w1, ready_w2 = ([set(), set()] for _ in range(4))
    for l in range(n_lane):
        queue_transpose(0, l)
    side.add(0, lambda: side.anchor_to(x_v[0:16, 0:LANES].astype(F32)))

    def arriving(l):
        if l % 2 == 0:
            side.add(0, wait, "x1%d" % l)
        queue_transpose(1, l)

    queue_input(0, arriving)
    side.add(0, wait, "wk0")
    side.add(0, side.anchor_to)
    queue_qkv_weights(1, range(3))
    side.flush()

    def after_step(n):
        if n == WAIT_AT[0]:
            side.add(WAIT_DELAY, lambda: None)
            side.add(0, wait, "wk1", "wq")
            queue_qkv_weights(1, range(3, 4))
            queue_qkv_weights(0, range(4))
        if n == WAIT_AT[1]:
            side.add(WAIT_DELAY, lambda: None)
            side.add(0, wait, "wv", "wo", "x2")
            queue_qkv_weights(2, range(4))
            for i in (2, 3):
                for l in range(n_lane):
                    queue_transpose(i, l)
            queue_input(1)
        if n == WAIT_AT[2]:
            queue_weights(wo, k_tile_of(wo_v), range(kd))

    for s in range(2):
        for n, part in enumerate((1, 0, 2)):
            side.tune("qkv"[part] + str(s))
            for c in range(4):
                wqkv.matmul(4 * part + c, rhs_s[s], ready_qkv[s], functools.partial(emit, part, s, c))
                after_step(12 * s + 4 * n + c)
            if (n, s) == (1, 1):
                side.add_urgent(150, range_check)
    side.flush()

    n_units = n_tiles * n_pairs

    def store_pair(p, i, first, second):
        inv = 1.0 / jnp.where(low4, second[0:8], first[16:24])
        swapped = jnp.concatenate([inv[4:8], inv[0:4]], axis=0)
        inv1, inv2 = jnp.where(low4, swapped, inv), jnp.where(low4, inv, swapped)
        ot_s[i, p] = jnp.concatenate(
            [first[0:8] * inv1, first[8:16] * inv1, jnp.where(low4, first[16:24] * inv1, second[0:8] * inv2),
             second[8:16] * inv2, second[16:24] * inv2], axis=0)

    def store_raw(unit):
        store_pair(unit % n_pairs, unit // n_pairs, raw_s[0], raw_s[1])

    def packed_attention(first_unit, n_steps, per_step):
        n_blk = seq // KEY_BLK
        items = [(u, t) for u in range(per_step) for t in range(n_blk)]

        def step(it, carry):
            unit0 = first_unit + it * per_step
            if first_unit > 0:
                store_raw(unit0 - 1)

            def locate(u):
                return (unit0 + u) // n_pairs, (unit0 + u) % n_pairs

            scores, probs, acc = {}, {}, {}
            for n in range(len(items) + max(LAGS)):
                if n < len(items):
                    u, t = items[n]
                    i, p = locate(u)
                    scores[n] = jnp.concatenate(
                        [_dot(k_s[p // 2, pl.ds(t * KEY_BLK + sum(SUBS[:j]), r), pl.ds(64 * (u % 2), 64)], q_s[i, p])
                         for j, r in enumerate(SUBS)], axis=0)
                if 1 <= n <= len(items):
                    s = scores.pop(n - 1)
                    probs[n - 1] = [jnp.exp2(score(s)).astype(BF16) for score in (_first_score, _second_score)]
                for h in (1, 0):
                    m = n - LAGS[h]
                    if 0 <= m < len(items):
                        u, t = items[m]
                        i, p = locate(u)
                        r = _dot(v_s[p, pl.ds(24 * h, 24), pl.ds(t * KEY_BLK, KEY_BLK)], probs[m][h])
                        acc[u, h] = r if t == 0 else acc[u, h] + r
                        if t == n_blk - 1 and u == per_step - 1:
                            raw_s[h] = acc[u, h]
                m = n - max(LAGS)
                if 0 <= m < len(items) and items[m][1] == n_blk - 1 and items[m][0] < per_step - 1:
                    u = items[m][0]
                    i, p = locate(u)
                    store_pair(p, i, acc[u, 0], acc[u, 1])
            return carry

        if n_steps == 1:
            step(0, 0)
        else:
            lax.fori_loop(0, n_steps, step, 0)

    wait("w1", "w2", "b1", "b2")
    for loop in LOOPS:
        pl.when(packed[0] == 1)(functools.partial(packed_attention, *loop))

    @pl.when(packed[0] != 1)
    def _():
        row = lax.broadcasted_iota(I32, (128, TOK), 0)

        def head(it, carry):
            unit, h = it // 2, it % 2
            i, p = unit // n_pairs, unit % n_pairs
            w = q_s[i, p].astype(F32)
            row0 = (p % 2) * 64 + 40 * h
            w = jnp.where((row >= row0) & (row < row0 + 24), jnp.concatenate([w, w], axis=0), 0.0)
            s = _dot(k_s[p // 2], w.astype(BF16)) * jnp.where(h == 0, 1.0 / HI_SCALE, 1.0)
            e = jnp.exp2(s - jnp.max(s, axis=0, keepdims=True)).astype(BF16)
            raw_s[h] = _dot(v_s[p, pl.ds(pl.multiple_of(24 * h, 8), 24), :], e)

            @pl.when(h == 1)
            def _():
                store_raw(unit)

            return carry

        lax.fori_loop(0, 2 * n_units, head, 0)

    side.anchor_to()
    store_raw(n_units - 1)

    def attn_rows(i, row, n, l):
        return jnp.concatenate([ot_s[side.zero() + i, r // pr, pl.ds(r % pr, 8), _blk(l)]
                                for r in range(row, row + n, 8)], axis=0)

    def add_residual(i, row0, y):
        rows = pl.ds(row0, ROWS)
        h = jnp.concatenate([xt[rows, :] for xt in xt_s[i]], axis=1) + y
        h_s[i][rows, :] = h
        accumulate(("h", i), h)

    def activate(s, c, l, y):
        a = []
        for j in range(4):
            bias = b1_s[pl.ds(c * LANES + (j // 2) * ROWS, ROWS), :]
            t = jnp.maximum(y[j][:, l * LANES:(l + 1) * LANES] + bias, 0.0)
            a.append(t * t)
        for j, v in enumerate(w2.rhs_ops(*a)):
            hid_s[s][j * w2.half + c // 2, l, pl.ds(c % 2 * ROWS, ROWS), :] = v.astype(BF16)

    def finish(i, c, top, bot):
        y = jnp.concatenate([top, bot], axis=0) + jnp.concatenate([b2_s[_blk(c), :]] * n_lane, axis=1)
        out_v[pl.ds(i * TOK, TOK), _blk(c)] = (h_s[i][_blk(c), :] + y).T.astype(BF16)

    parts = ((pl.ds(0, 2 * TOK), pl.ds(0, dim)), (pl.ds(2 * TOK, 2 * TOK), pl.ds(0, dim - LANES)),
             (pl.ds(2 * TOK, 2 * TOK), _blk(kd - 1)))
    out_cp = [pltpu.make_async_copy(out_v.at[rows, cols], out_hbm.at[0, rows, cols], out_sem.at[j])
              for j, (rows, cols) in enumerate(parts)]

    def send(cp, earlier):
        cp.start()
        earlier.wait()

    for s in range(2):
        x0, x1 = [functools.partial(attn_rows, i) for i in (2 * s, 2 * s + 1)]
        wo.queue_rhs(rhs_s[2 + s], ready_wo[s], x0, x1, 28)
    side.add(200, bias_column, b1_v, b1_s)
    queue_weights(w1, k_tile_of(w1_v), range(W1_EARLY))
    for s in range(2):
        side.tune("wo%d" % s)
        for c in range(kd):
            wo.matmul(c, rhs_s[2 + s], ready_wo[s], lambda half, tile, y: side.add_urgent(
                50, add_residual, 2 * s + tile, c * LANES + half * ROWS, y))
        for i in (2 * s, 2 * s + 1):
            side.add_urgent(10, moments, ("h", i))
        x0, x1 = [normalized(lambda rows, l, i=i: h_s[i][rows, _blk(l)],
                             lambda l, i=i: [t[:, l * LANES:(l + 1) * LANES] for t in stats["h", i]])
                  for i in (2 * s, 2 * s + 1)]
        w1.queue_rhs(rhs_s[s], ready_w1[s], x0, x1, 34)
        if s == 0:
            queue_weights(w1, k_tile_of(w1_v), range(W1_EARLY, kf))
        else:
            side.add(80, bias_column, b2_v, b2_s)
            queue_weights(w2, w2_k_tile, range(kd))
    for s in range(2):
        side.tune("w1%d" % s)
        for c in range(kf):
            y = {}
            w1.matmul(c, rhs_s[s], ready_w1[s], lambda half, tile, value: y.update({2 * half + tile: value}))
            for l in range(n_lane):
                side.add_urgent(42, activate, s, c, l, y)
            if c % 2:
                side.add_urgent(0, ready_w2[s].update, range(c // 2, 7 * w2.half, w2.half))
        side.tune("w2%d" % s)
        for c in range(kd):
            bottom = {}

            def collect(half, tile, value):
                if half:
                    bottom[tile] = value
                else:
                    side.add_urgent(70, finish, 2 * s + tile, c, value, bottom[tile])

            w2.matmul(c, hid_s[s], ready_w2[s], collect)
            if (s, c) in ((1, 0), (1, kd - 2)):
                side.add_urgent(100, lambda: None)
                side.add_urgent(0, send, *((out_cp[0], copy["fence"]) if c == 0 else (out_cp[1], out_cp[0])))
    side.flush()
    out_cp[2].start()
    out_cp[1].wait()
    out_cp[2].wait()


@jax.jit
def pallas_sequential_preLN__softmax_full_mha__dense_activation_squared_relu__prompt_kernel(
    A_x: jax.Array,
    A_wqkv: jax.Array,
    A_wo: jax.Array,
    B_x: jax.Array,
    B_w1: jax.Array,
    B_b1: jax.Array,
    B_w2: jax.Array,
    B_b2: jax.Array,
):
    del B_x
    _, seq, dim = A_x.shape
    ff = B_w1.shape[1]
    assert (seq, dim, ff) == (4 * TOK, 20 * N_HEADS, 12 * LANES), "the tiling is laid out for these shapes"
    n_pairs, n_tiles, n_lane = N_HEADS // 2, seq // TOK, TOK // LANES
    pr = 2 * dim // N_HEADS
    kd, kf = dim // LANES, ff // LANES
    ops_d, ops_f = 7 * (kd // 2) + 2, 7 * (kf // 2)
    any_spec = pl.BlockSpec(memory_space=pl.ANY)
    return pl.pallas_call(
        _block_kernel,
        out_shape=jax.ShapeDtypeStruct(A_x.shape, A_x.dtype),
        in_specs=[any_spec] * 7,
        out_specs=any_spec,
        scratch_shapes=[
            pltpu.VMEM((seq, dim), BF16),
            pltpu.VMEM((dim, 3 * dim), BF16),
            pltpu.VMEM((dim, dim), BF16),
            pltpu.VMEM((dim, ff), BF16),
            pltpu.VMEM((ff, dim), BF16),
            [pltpu.VMEM((kd, dim, LANES), F32)] * 3,
            [pltpu.VMEM((ops_d, 2 * pr, LANES), BF16)] * (3 * n_pairs // 4),
            [pltpu.VMEM((ops_d, ROWS, LANES), BF16)] * kd,
            [pltpu.VMEM((ops_d, ROWS, LANES), BF16)] * kf,
            [pltpu.VMEM((ops_f, ROWS, LANES), BF16)] * kd,
            pltpu.VMEM((ff, LANES), F32),
            pltpu.VMEM((dim, LANES), F32),
            [[pltpu.VMEM((dim, LANES), F32)] * n_lane] * n_tiles,
            [pltpu.VMEM((dim, TOK), F32)] * n_tiles,
            [pltpu.VMEM((ops_d, n_lane, LANES, LANES), BF16)] * 4,
            [pltpu.VMEM((ops_f, n_lane, LANES, LANES), BF16)] * 2,
            pltpu.VMEM((n_pairs // 2, seq, LANES), BF16),
            pltpu.VMEM((n_tiles, n_pairs, 64, TOK), BF16),
            pltpu.VMEM((n_pairs, 48, seq), F32),
            pltpu.VMEM((2, 24, TOK), F32),
            pltpu.VMEM((n_tiles, n_pairs, pr, TOK), F32),
            pltpu.VMEM((seq, dim), BF16),
            pltpu.VMEM((ff,), BF16),
            pltpu.VMEM((dim,), BF16),
            pltpu.VMEM((23 * 256,), BF16),
            pltpu.SemaphoreType.DMA((14,)),
            pltpu.SemaphoreType.DMA((3,)),
        ],
        compiler_params=pltpu.CompilerParams(vmem_limit_bytes=110 * 2 ** 20),
        name="fused_block",
    )(A_x, A_wqkv, A_wo, B_w1, B_b1, B_w2, B_b2)
```
